```python
import os as _os
_os.environ.setdefault("JAX_PLATFORMS", "cpu")
import jax
import jax.numpy as jnp

def _softmax(x, axis=-1):
    return jax.nn.softmax(x, axis=axis)
def _gelu(x):
    return jax.nn.gelu(x, approximate=True)
def _silu(x):
    return jax.nn.silu(x)
def _sigmoid(x):
    return jax.nn.sigmoid(x)
def _layernorm(x, axis=-1, eps=1e-5):
    m = jnp.mean(x, axis=axis, keepdims=True)
    v = jnp.var(x, axis=axis, keepdims=True)
    return (x - m) / jnp.sqrt(v + eps)
def _scatter_add(tgt, idx, src, axis=0):
    return tgt.at[idx].add(src)
def _segment_sum(src, seg, n):
    return jax.ops.segment_sum(src, seg, n)
class _Rng:
    def __init__(self, key):
        self._k = key
    def _next(self):
        self._k, sub = jax.random.split(self._k)
        return sub
    def normal(self, shape):
        return jax.random.normal(self._next(), shape, dtype=jnp.bfloat16)
    def randint(self, lo, hi, shape):
        return jax.random.randint(self._next(), shape, lo, hi, dtype=jnp.int32)
    def uniform(self, shape, lo=0.0, hi=1.0):
        return jax.random.uniform(self._next(), shape, jnp.bfloat16, lo, hi)
    def permutation(self, n):
        return jax.random.permutation(self._next(), n)


kernel_name = 'parallel_sum__softmax_full_mha__moe_arch_mod__prompt'

def setup_inputs():
    _rng = _Rng(jax.random.key(int.from_bytes(__import__("os").urandom(4), "little")))
    _w = (lambda a: (lambda t: t.astype(jnp.bfloat16) if jnp.issubdtype(t.dtype, jnp.floating) else t)(jnp.asarray(a)))
    def _A_setup():
        B, S, D = 1, 2048, 512
        return {
            "x": _w((lambda *s: _rng.normal(s) * 0.05)(B, S, D)),
            "wqkv": _w((lambda *s: _rng.normal(s) * 0.1)(D, 3 * D)),
            "wo": _w((lambda *s: _rng.normal(s) * 0.05)(D, D)),
        }
    _A_in = _A_setup()

    def _B_setup():
        B, S, D, F, C = 1, 2048, 512, 1792, 1
        return {
            "x": _w((lambda *s: _rng.normal(s) * 0.05)(B, S, D)),
            "w_r": _w((lambda *s: _rng.normal(s) * 1.6)(D)),
            "w_gate": _w((lambda *s: _rng.normal(s) * 0.1)(D, F)),
            "w_up": _w((lambda *s: _rng.normal(s) * 0.1)(D, F)),
            "w_down": _w((lambda *s: _rng.normal(s) * 0.1)(F, D)),
        }
    _B_in = _B_setup()

    return {
        "A_x": _A_in["x"],
        "A_wqkv": _A_in["wqkv"],
        "A_wo": _A_in["wo"],
        "B_x": _B_in["x"],
        "B_w_r": _B_in["w_r"],
        "B_w_gate": _B_in["w_gate"],
        "B_w_up": _B_in["w_up"],
        "B_w_down": _B_in["w_down"],
    }

def reference(A_x, A_wqkv, A_wo, B_x, B_w_r, B_w_gate, B_w_up, B_w_down):
    def _A_ref(x, wqkv, wo):
        B, S, D = x.shape
        H = 32; Dh = D // H
        qkv = (lambda x, *d: x.transpose(*d))((x @ wqkv).reshape(B, S, 3, H, Dh), 2, 0, 3, 1, 4)
        q, k, v = qkv[0], qkv[1], qkv[2]
        scale = Dh ** -0.5
        scores = jnp.einsum("bhqd,bhkd->bhqk", q, k) * scale
        p = _softmax(scores, axis=-1)
        o = jnp.einsum("bhqk,bhkd->bhqd", p, v)
        return (lambda x, *d: x.transpose(*d))(o, 0, 2, 1, 3).reshape(B, S, D) @ wo

    def _B_ref(x, w_r, w_gate, w_up, w_down):
        B, S, D = x.shape
        C = 1
        r = x @ w_r
        idx = jnp.argsort(-r, axis=-1)[:, :C]
        idx_e = jnp.repeat(idx.reshape(B, C, 1), D, axis=2)
        x_sel = jnp.take_along_axis(x, idx_e, axis=1)
        g = _silu(x_sel @ w_gate)
        u = x_sel @ w_up
        y = (g * u) @ w_down
        r_sel = _sigmoid(jnp.take_along_axis(r, idx, axis=1))
        y = y * r_sel.reshape(B, C, 1)
        b_off = (jnp.arange(B) * S).reshape(B, 1)
        flat_idx = (idx + b_off).reshape(B * C)
        zero = (x * 0.0).reshape(B * S, D)
        upd = _scatter_add(zero, flat_idx, y.reshape(B * C, D), axis=0)
        return x + upd.reshape(B, S, D)

    x = A_x
    xn = _layernorm(x, axis=-1)
    return x + _A_ref(xn, A_wqkv, A_wo) + _B_ref(xn, B_w_r, B_w_gate, B_w_up, B_w_down)
```

```python
import functools
import math

import jax
import jax.numpy as jnp
import jax.experimental.pallas as pl
import jax.experimental.pallas.tpu as pltpu

H = 32
TQ = 512
CK = 256
VR = 32

_NT = (((1,), (1,)), ((), ()))


def _bf16r(x):
    return x.astype(jnp.bfloat16).astype(jnp.float32)


def _kernel(x_ref, wqkv_ref, wo_ref, wr_ref, wg_hbm, wu_hbm, wd_hbm, o_ref,
            xn_ref, q_ref, k_ref, vt_ref, s0_ref, s1_ref, m0_ref, m1_ref, ot_ref,
            wg_ref, wu_ref, wd_ref, sems):
    S, D = x_ref.shape
    Dh = D // H
    G = D // 128
    HPG = 128 // Dh
    NQ = S // TQ
    NC = S // CK
    T = H * NQ

    cps = [pltpu.make_async_copy(wg_hbm, wg_ref, sems.at[0]),
           pltpu.make_async_copy(wu_hbm, wu_ref, sems.at[1]),
           pltpu.make_async_copy(wd_hbm, wd_ref, sems.at[2])]
    for c in cps:
        c.start()

    xf = x_ref[...].astype(jnp.float32)
    mean = jnp.mean(xf, axis=-1, keepdims=True)
    cen = xf - mean
    var = jnp.mean(cen * cen, axis=-1, keepdims=True)
    eps = 1.0013580322265625e-05
    den = _bf16r(jnp.sqrt(_bf16r(_bf16r(var) + eps)))
    xn = (_bf16r(xf - _bf16r(mean)) / den).astype(jnp.bfloat16)
    xn_ref[...] = xn

    qscale = (Dh ** -0.5) * math.log2(math.e)
    for g in range(G):
        wq = wqkv_ref[:, g * 128:(g + 1) * 128]
        q = jnp.dot(xn, wq, preferred_element_type=jnp.float32)
        q_ref[g] = (q * qscale).astype(jnp.bfloat16)
        wk = wqkv_ref[:, D + g * 128:D + (g + 1) * 128]
        k_ref[g] = jnp.dot(xn, wk, preferred_element_type=jnp.float32).astype(jnp.bfloat16)
    wvt = wqkv_ref[:, 2 * D:3 * D].astype(jnp.float32).T.astype(jnp.bfloat16)
    vt = jax.lax.dot_general(wvt, xn, _NT, preferred_element_type=jnp.float32)
    row = jax.lax.broadcasted_iota(jnp.int32, (VR - Dh, S), 0)
    tail = jnp.where(row == 0, 1.0, 0.0).astype(jnp.float32)
    for h in range(H):
        vt_ref[h] = jnp.concatenate([vt[h * Dh:(h + 1) * Dh], tail], axis=0).astype(jnp.bfloat16)

    lane_head = jax.lax.broadcasted_iota(jnp.int32, (TQ, 128), 1) // Dh

    def masked_q(t):
        h = t // NQ
        qi = t % NQ
        g = h // HPG
        qt = q_ref[g, pl.ds(pl.multiple_of(qi * TQ, TQ), TQ), :]
        return g, jnp.where(lane_head == (h % HPG), qt, jnp.zeros_like(qt))

    def a_chunk(g, qm, c, s_ref, m):
        kc = k_ref[g, c * CK:(c + 1) * CK, :]
        s = jax.lax.dot_general(kc, qm, _NT, preferred_element_type=jnp.float32)
        s_ref[c * CK:(c + 1) * CK, :] = s
        mc = jnp.max(s.reshape(CK // 8, 8, TQ), axis=0)
        return mc if m is None else jnp.maximum(m, mc)

    def b_chunk(h, c, s_ref, m, acc):
        p = jnp.exp2(s_ref[c * CK:(c + 1) * CK, :] - m).astype(jnp.bfloat16)
        pv = jnp.dot(vt_ref[h, :, c * CK:(c + 1) * CK], p, preferred_element_type=jnp.float32)
        return pv if acc is None else acc + pv

    def step(t_b, sb_ref, mb_ref, t_a, sa_ref, ma_ref):
        if t_a is not None:
            g, qm = masked_q(t_a)
        if t_b is not None:
            hb = t_b // NQ
            mb = mb_ref[...]
        ma = None
        acc = None
        for c in range(NC):
            if t_a is not None:
                ma = a_chunk(g, qm, c, sa_ref, ma)
            if t_b is not None:
                acc = b_chunk(hb, c, sb_ref, mb, acc)
        if t_a is not None:
            ma_ref[...] = jnp.max(ma, axis=0, keepdims=True)
        if t_b is not None:
            o = acc[:Dh] / acc[Dh:Dh + 1]
            ot_ref[t_b % NQ, hb] = o

    step(None, None, None, 0, s0_ref, m0_ref)

    def body(i, carry):
        t = 2 * i
        step(t, s0_ref, m0_ref, t + 1, s1_ref, m1_ref)
        step(t + 1, s1_ref, m1_ref, t + 2, s0_ref, m0_ref)
        return carry

    jax.lax.fori_loop(0, T // 2 - 1, body, 0)
    step(T - 2, s0_ref, m0_ref, T - 1, s1_ref, m1_ref)
    step(T - 1, s1_ref, m1_ref, None, None, None)

    xn = xn_ref[...]
    wr8 = jnp.broadcast_to(wr_ref[...], (8, D))
    r = jax.lax.dot_general(wr8, xn, _NT, preferred_element_type=jnp.float32)
    r = _bf16r(r)
    rmax = jnp.max(r, axis=-1, keepdims=True)
    col = jax.lax.broadcasted_iota(jnp.int32, (8, S), 1)
    idx = jnp.min(jnp.where(r == rmax, col, S), axis=-1, keepdims=True)
    onehot = jnp.where(col == idx, 1.0, 0.0).astype(jnp.bfloat16)
    x_sel = jnp.dot(onehot, xn, preferred_element_type=jnp.float32).astype(jnp.bfloat16)
    for c in cps:
        c.wait()
    gate = jnp.dot(x_sel, wg_ref[...], preferred_element_type=jnp.float32)
    up = jnp.dot(x_sel, wu_ref[...], preferred_element_type=jnp.float32)
    hmid = (gate * jax.nn.sigmoid(gate) * up).astype(jnp.bfloat16)
    y = jnp.dot(hmid, wd_ref[...], preferred_element_type=jnp.float32)
    y = y * jax.nn.sigmoid(rmax)
    y1 = y[0:1]
    idx1 = idx[0:1]

    wo = wo_ref[...]
    for qi in range(NQ):
        ot = ot_ref[qi].reshape(D, TQ)
        o = ot.T.astype(jnp.bfloat16)
        att = jnp.dot(o, wo, preferred_element_type=jnp.float32)
        rows = slice(qi * TQ, (qi + 1) * TQ)
        rid = jax.lax.broadcasted_iota(jnp.int32, (TQ, D), 0) + qi * TQ
        upd = jnp.where(rid == idx1, y1, 0.0)
        res = (x_ref[rows, :].astype(jnp.float32) + att) + (xn_ref[rows, :].astype(jnp.float32) + upd)
        o_ref[rows, :] = res.astype(o_ref.dtype)


@jax.jit
def pallas_parallel_sum__softmax_full_mha__moe_arch_mod__prompt_kernel(
    A_x: jax.Array,
    A_wqkv: jax.Array,
    A_wo: jax.Array,
    B_x: jax.Array,
    B_w_r: jax.Array,
    B_w_gate: jax.Array,
    B_w_up: jax.Array,
    B_w_down: jax.Array,
):
    B, S, D = A_x.shape
    assert B == 1
    F = B_w_gate.shape[1]
    Dh = D // H
    bf = jnp.bfloat16
    vmem = pl.BlockSpec(memory_space=pltpu.VMEM)
    hbm = pl.BlockSpec(memory_space=pl.ANY)
    out = pl.pallas_call(
        _kernel,
        out_shape=jax.ShapeDtypeStruct((S, D), A_x.dtype),
        in_specs=[vmem, vmem, vmem, vmem, hbm, hbm, hbm],
        out_specs=vmem,
        scratch_shapes=[
            pltpu.VMEM((S, D), bf),
            pltpu.VMEM((D // 128, S, 128), bf),
            pltpu.VMEM((D // 128, S, 128), bf),
            pltpu.VMEM((H, VR, S), bf),
            pltpu.VMEM((S, TQ), jnp.float32),
            pltpu.VMEM((S, TQ), jnp.float32),
            pltpu.VMEM((1, TQ), jnp.float32),
            pltpu.VMEM((1, TQ), jnp.float32),
            pltpu.VMEM((S // TQ, H, Dh, TQ), jnp.float32),
            pltpu.VMEM((D, F), bf),
            pltpu.VMEM((D, F), bf),
            pltpu.VMEM((F, D), bf),
            pltpu.SemaphoreType.DMA((3,)),
        ],
        compiler_params=pltpu.CompilerParams(vmem_limit_bytes=100 * 1024 * 1024),
    )(A_x.reshape(S, D), A_wqkv, A_wo, B_w_r.reshape(1, D), B_w_gate, B_w_up, B_w_down)
    return out.reshape(B, S, D)
```

```python
import functools
import math

import jax
import jax.numpy as jnp
import jax.experimental.pallas as pl
import jax.experimental.pallas.tpu as pltpu

H = 32
TQ = 512
CK = 128
SKEW = 1
U = 4
KW = 32
LAG = 2

_NT = (((1,), (1,)), ((), ()))


def _bf16r(x):
    return x.astype(jnp.bfloat16).astype(jnp.float32)


def _kernel(x_hbm, wqkv_hbm, wo_hbm, wr_ref, wg_hbm, wu_hbm, wd_hbm, o_hbm,
            x_ref, wqkv_ref, wo_ref, o_ref, xn_ref, q_ref, k_ref, vt_ref,
            s0_ref, s1_ref, m0_ref, m1_ref, pm_ref, ot_ref, r_ref,
            wg_ref, wu_ref, wd_ref, sems):
    S, D = x_ref.shape
    Dh = D // H
    G = D // 128
    HPG = 128 // Dh
    NQ = S // TQ
    NC = S // CK
    T = H * NQ

    x_cps = [pltpu.make_async_copy(x_hbm.at[pl.ds(i * TQ, TQ)], x_ref.at[pl.ds(i * TQ, TQ)], sems.at[i])
             for i in range(NQ)]
    w_cps = [pltpu.make_async_copy(wqkv_hbm.at[:, pl.ds(i * D, D)], wqkv_ref.at[i], sems.at[NQ + i])
             for i in range(3)]
    f_cps = [pltpu.make_async_copy(wg_hbm, wg_ref, sems.at[NQ + 3]),
             pltpu.make_async_copy(wu_hbm, wu_ref, sems.at[NQ + 4]),
             pltpu.make_async_copy(wd_hbm, wd_ref, sems.at[NQ + 5])]
    wo_cp = pltpu.make_async_copy(wo_hbm, wo_ref, sems.at[NQ + 6])

    qscale = (Dh ** -0.5) * math.log2(math.e)
    eps = 1.0013580322265625e-05

    def layernorm(qi):
        rows = slice(qi * TQ, (qi + 1) * TQ)
        xf = x_ref[rows, :].astype(jnp.float32)
        mean = jnp.mean(xf, axis=-1, keepdims=True)
        cen = xf - mean
        var = jnp.mean(cen * cen, axis=-1, keepdims=True)
        den = _bf16r(jnp.sqrt(_bf16r(_bf16r(var) + eps)))
        xn_ref[rows, :] = (_bf16r(xf - _bf16r(mean)) / den).astype(jnp.bfloat16)

    def kproj(qi):
        rows = slice(qi * TQ, (qi + 1) * TQ)
        xn = xn_ref[rows, :]
        for g in range(G):
            kg = jnp.dot(xn, wqkv_ref[1, :, g * 128:(g + 1) * 128],
                         preferred_element_type=jnp.float32).astype(jnp.bfloat16)
            for hh in range(128 // KW):
                k_ref[g * (128 // KW) + hh, rows, :] = kg[:, hh * KW:(hh + 1) * KW]

    def qvproj(qi, wqt, wvt):
        rows = slice(qi * TQ, (qi + 1) * TQ)
        xn = xn_ref[rows, :]
        qt = jax.lax.dot_general(wqt, xn, _NT, preferred_element_type=jnp.float32)
        q_ref[qi] = (qt[:D] * qscale).astype(jnp.bfloat16).reshape(D // KW, KW, TQ)
        r_ref[:, rows] = _bf16r(qt[D:D + 8])
        vt = jax.lax.dot_general(wvt, xn, _NT, preferred_element_type=jnp.float32)
        vt_ref[:, :, rows] = vt.reshape(H, Dh, TQ).astype(jnp.bfloat16)

    x_cps[0].start()
    w_cps[1].start()
    x_cps[1].start()
    x_cps[0].wait()
    w_cps[0].start()
    w_cps[2].start()
    for c in x_cps[2:]:
        c.start()
    layernorm(0)
    w_cps[1].wait()
    x_cps[1].wait()
    kproj(0)
    layernorm(1)
    w_cps[0].wait()
    w_cps[2].wait()
    for c in x_cps[2:]:
        c.wait()
    for c in f_cps:
        c.start()
    wo_cp.start()
    wr16 = jnp.broadcast_to(wr_ref[...].reshape(1, D).astype(jnp.float32), (16, D))
    wqt = jnp.concatenate([wqkv_ref[0].astype(jnp.float32).T, wr16], axis=0).astype(jnp.bfloat16)
    wvt = wqkv_ref[2].astype(jnp.float32).T.astype(jnp.bfloat16)
    kproj(1)
    for qi in range(NQ):
        if qi + 2 < NQ:
            layernorm(qi + 2)
        qvproj(qi, wqt, wvt)
        if qi + 2 < NQ:
            kproj(qi + 2)

    st = {}
    FB = 256
    F = wg_ref.shape[1]

    def sel_piece():
        r = r_ref[...]
        rmax = jnp.max(r, axis=-1, keepdims=True)
        col = jax.lax.broadcasted_iota(jnp.int32, (8, S), 1)
        idx = jnp.min(jnp.where(r == rmax, col, S - 1))
        st["rmax"] = rmax[0:1]
        st["idx1"] = idx
        blk = xn_ref[pl.ds(pl.multiple_of((idx // 16) * 16, 16), 16), :]
        rid = jax.lax.broadcasted_iota(jnp.int32, (16, D), 0)
        st["x_sel"] = jnp.where(rid == idx % 16, blk, jnp.zeros_like(blk))

    def gu_piece(j):
        cols = slice(j * FB, (j + 1) * FB)
        gate = jnp.dot(st["x_sel"], wg_ref[:, cols], preferred_element_type=jnp.float32)
        up = jnp.dot(st["x_sel"], wu_ref[:, cols], preferred_element_type=jnp.float32)
        st[("h", j)] = (gate * jax.nn.sigmoid(gate) * up).astype(jnp.bfloat16)

    def down_piece(j):
        y = jnp.dot(st[("h", j)], wd_ref[j * FB:(j + 1) * FB, :], preferred_element_type=jnp.float32)
        st["y"] = y if j == 0 else st["y"] + y
        if j == F // FB - 1:
            st["y1"] = jnp.sum(st["y"], axis=0, keepdims=True) * jax.nn.sigmoid(st["rmax"])

    moe_pieces = ([sel_piece]
                  + [None]
                  + [functools.partial(gu_piece, j) for j in range(F // FB)]
                  + [None]
                  + [functools.partial(down_piece, j) for j in range(F // FB)])

    o_cps = []

    def outproj(qi):
        idx1, y1 = st["idx1"], st["y1"]
        ot = ot_ref[qi].reshape(D, TQ)
        o = ot.T.astype(jnp.bfloat16)
        att = jnp.dot(o, wo_ref[...], preferred_element_type=jnp.float32)
        rows = slice(qi * TQ, (qi + 1) * TQ)
        rid = jax.lax.broadcasted_iota(jnp.int32, (TQ, D), 0) + qi * TQ
        upd = jnp.where(rid == idx1, y1, 0.0)
        res = (x_ref[rows, :].astype(jnp.float32) + att) + (xn_ref[rows, :].astype(jnp.float32) + upd)
        o_ref[rows, :] = res.astype(o_ref.dtype)
        ocp = pltpu.make_async_copy(o_ref.at[pl.ds(qi * TQ, TQ)], o_hbm.at[pl.ds(qi * TQ, TQ)], sems.at[qi])
        ocp.start()
        o_cps.append(ocp)

    def a_chunk(h, qm, c, s_ref, m):
        kc = k_ref[h, c * CK:(c + 1) * CK, :]
        s = jnp.dot(kc, qm, preferred_element_type=jnp.float32)
        s_ref[c * CK:(c + 1) * CK, :] = s
        mc = jnp.max(s.reshape(CK // 8, 8, TQ), axis=0)
        return (mc if m is None else jnp.maximum(m, mc)), s[0:8]

    def b_chunk(h, c, s_ref, m, acc, tok):
        m = jnp.broadcast_to(m, (8, TQ))
        if tok is not None:
            m = jnp.maximum(m, jnp.minimum(m, tok))
        p = jnp.exp2(s_ref[c * CK:(c + 1) * CK, :].reshape(CK // 8, 8, TQ) - m[None]).reshape(CK, TQ)
        l = None
        for kt in range(CK // 128):
            lt = None
            for r in reversed(range(8)):
                a = p[kt * 128 + r * 16: kt * 128 + r * 16 + 8] + p[kt * 128 + r * 16 + 8: kt * 128 + r * 16 + 16]
                lt = a if lt is None else lt + a
            l = lt if l is None else l + lt
        pv = jnp.dot(vt_ref[h, :, c * CK:(c + 1) * CK], p.astype(jnp.bfloat16), preferred_element_type=jnp.float32)
        return (pv, l) if acc is None else (acc[0] + pv, acc[1] + l)

    s_refs = (s0_ref, s1_ref)
    m_refs = (m0_ref, m1_ref)

    def group(t, first=False, last=False, hooks=None):
        qcache = {}
        pmax = {}
        binfo = {}
        acc = {}
        toks = []
        n_b = 0 if first else U * NC
        a_lo = 0 if first else NC + SKEW
        a_hi = (NC + SKEW) if first else (U * NC if last else (U + 1) * NC + SKEW)
        n = max(n_b, a_hi - a_lo)
        for i in range(n):
            if hooks and i in hooks:
                hooks[i]()
            ja = a_lo + i
            if ja < a_hi:
                u, c = ja // NC, ja % NC
                if u not in qcache:
                    ha = (t + u) % H
                    hpk = KW // Dh
                    qg = q_ref[(t + u) // H, ha // hpk]
                    if hpk > 1:
                        rh = jax.lax.broadcasted_iota(jnp.int32, (KW, TQ), 0) // Dh
                        qg = jnp.where(rh == ha % hpk, qg, jnp.zeros_like(qg))
                    qcache[u] = (ha // hpk, qg)
                    pmax[u] = pm_ref[...] if c > 0 else None
                ha, qm = qcache[u]
                pmax[u], tk = a_chunk(ha, qm, c, s_refs[u % 2], pmax[u])
                toks.append(tk)
                if c == NC - 1:
                    m_refs[u % 2][...] = jnp.max(pmax[u], axis=0, keepdims=True)
                elif ja == a_hi - 1:
                    pm_ref[...] = pmax[u]
            if i < n_b:
                u, c = i // NC, i % NC
                if u not in binfo:
                    binfo[u] = ((t + u) % H, m_refs[u % 2][...])
                    acc[u] = None
                hb, mb = binfo[u]
                acc[u] = b_chunk(hb, c, s_refs[u % 2], mb, acc[u],
                                 toks[i - LAG] if 0 <= i - LAG < len(toks) else None)
                if c == NC - 1:
                    o = acc[u][0] / jnp.sum(acc[u][1], axis=0, keepdims=True)
                    ot_ref[(t + u) // H, hb] = o

    group(0, first=True)

    def body(i, carry):
        group(U * i)
        return carry

    jax.lax.fori_loop(0, T // U - 1, body, 0)
    for c in f_cps:
        c.wait()
    wo_cp.wait()
    hooks = {}
    for i, pc in enumerate(moe_pieces):
        if pc is not None:
            hooks[1 + i] = pc
    for qi in range(NQ - 1):
        hooks[(U - 1) * NC - SKEW + qi * 5] = functools.partial(outproj, qi)
    group(T - U, last=True, hooks=hooks)
    outproj(NQ - 1)
    for c in o_cps:
        c.wait()


@jax.jit
def pallas_parallel_sum__softmax_full_mha__moe_arch_mod__prompt_kernel(
    A_x: jax.Array,
    A_wqkv: jax.Array,
    A_wo: jax.Array,
    B_x: jax.Array,
    B_w_r: jax.Array,
    B_w_gate: jax.Array,
    B_w_up: jax.Array,
    B_w_down: jax.Array,
):
    B, S, D = A_x.shape
    assert B == 1
    F = B_w_gate.shape[1]
    Dh = D // H
    bf = jnp.bfloat16
    vmem = pl.BlockSpec(memory_space=pltpu.VMEM)
    hbm = pl.BlockSpec(memory_space=pl.ANY)
    out = pl.pallas_call(
        _kernel,
        out_shape=jax.ShapeDtypeStruct((S, D), A_x.dtype),
        in_specs=[hbm, hbm, hbm, vmem, hbm, hbm, hbm],
        out_specs=hbm,
        scratch_shapes=[
            pltpu.VMEM((S, D), bf),
            pltpu.VMEM((3, D, D), bf),
            pltpu.VMEM((D, D), bf),
            pltpu.VMEM((S, D), bf),
            pltpu.VMEM((S, D), bf),
            pltpu.VMEM((S // TQ, D // KW, KW, TQ), bf),
            pltpu.VMEM((D // KW, S, KW), bf),
            pltpu.VMEM((H, Dh, S), bf),
            pltpu.VMEM((S, TQ), jnp.float32),
            pltpu.VMEM((S, TQ), jnp.float32),
            pltpu.VMEM((1, TQ), jnp.float32),
            pltpu.VMEM((1, TQ), jnp.float32),
            pltpu.VMEM((8, TQ), jnp.float32),
            pltpu.VMEM((S // TQ, H, Dh, TQ), jnp.float32),
            pltpu.VMEM((8, S), jnp.float32),
            pltpu.VMEM((D, F), bf),
            pltpu.VMEM((D, F), bf),
            pltpu.VMEM((F, D), bf),
            pltpu.SemaphoreType.DMA((7 + S // TQ,)),
        ],
        compiler_params=pltpu.CompilerParams(vmem_limit_bytes=100 * 1024 * 1024),
    )(A_x.reshape(S, D), A_wqkv, A_wo, B_w_r, B_w_gate, B_w_up, B_w_down)
    return out.reshape(B, S, D)
```

```python
import functools
import math

import jax
import jax.numpy as jnp
import jax.experimental.pallas as pl
import jax.experimental.pallas.tpu as pltpu

H = 32
TQ = 512
CK = 128
SKEW = 1
LAG = 2
NOFF = 6
PC_LO = 1
PC_HI = 13
PC_LAST = 12
QB_AT = 8
FB = 256

_NT = (((1,), (1,)), ((), ()))


def _bf16r(x):
    return x.astype(jnp.bfloat16).astype(jnp.float32)


def _kernel(x_hbm, wqkv_hbm, wo_hbm, wr_ref, wg_hbm, wu_hbm, wd_hbm, o_hbm,
            x_ref, wqkv_ref, wo_ref, o_ref, xn_ref, q_ref, k_ref, vt_ref,
            s0_ref, s1_ref, m0_ref, m1_ref, pm_ref, ot_ref, r_ref, kb_ref, qb0_ref, qb1_ref,
            wg_ref, wu_ref, wd_ref, sems):
    S, D = x_ref.shape
    F = wg_ref.shape[1]
    Dh = D // H
    G = D // 128
    HPG = 128 // Dh
    NQ = S // TQ
    NC = S // CK
    NL = TQ // 128
    assert PC_LO >= SKEW

    x_cps = [pltpu.make_async_copy(x_hbm.at[pl.ds(i * TQ, TQ)], x_ref.at[pl.ds(i * TQ, TQ)], sems.at[i])
             for i in range(NQ)]
    w_cps = [pltpu.make_async_copy(wqkv_hbm.at[:, pl.ds(i * D, D)], wqkv_ref.at[i], sems.at[NQ + i])
             for i in range(3)]
    f_cps = [pltpu.make_async_copy(wg_hbm, wg_ref, sems.at[NQ + 3]),
             pltpu.make_async_copy(wu_hbm, wu_ref, sems.at[NQ + 4]),
             pltpu.make_async_copy(wd_hbm, wd_ref, sems.at[NQ + 5])]
    wo_cp = pltpu.make_async_copy(wo_hbm, wo_ref, sems.at[NQ + 6])

    qscale = (Dh ** -0.5) * math.log2(math.e)
    eps = 1.0013580322265625e-05

    def layernorm(qi):
        rows = slice(qi * TQ, (qi + 1) * TQ)
        xf = x_ref[rows, :].astype(jnp.float32)
        mean = jnp.mean(xf, axis=-1, keepdims=True)
        cen = xf - mean
        var = jnp.mean(cen * cen, axis=-1, keepdims=True)
        den = _bf16r(jnp.sqrt(_bf16r(_bf16r(var) + eps)))
        xn_ref[rows, :] = (_bf16r(xf - _bf16r(mean)) / den).astype(jnp.bfloat16)

    def kproj(qi):
        xn = xn_ref[qi * TQ:(qi + 1) * TQ, :]
        for g in range(G):
            kg = jnp.dot(xn, wqkv_ref[1, :, g * 128:(g + 1) * 128],
                         preferred_element_type=jnp.float32).astype(jnp.bfloat16)
            for hh in range(HPG):
                k_ref[g * HPG + hh, qi * TQ // 2:(qi + 1) * TQ // 2, :] = pltpu.bitcast(
                    kg[:, hh * Dh:(hh + 1) * Dh], jnp.uint32)

    def qvproj(qi, wqt, wvt):
        rows = slice(qi * TQ, (qi + 1) * TQ)
        xn = xn_ref[rows, :]
        qt = jax.lax.dot_general(wqt, xn, _NT, preferred_element_type=jnp.float32)
        q_ref[qi] = (qt[:D] * qscale).astype(jnp.bfloat16).reshape(H, Dh, TQ)
        r_ref[:, rows] = _bf16r(qt[D:D + 8])
        vt = jax.lax.dot_general(wvt, xn, _NT, preferred_element_type=jnp.float32)
        vt_ref[:, :, rows] = vt.reshape(H, Dh, TQ).astype(jnp.bfloat16)

    x_cps[0].start()
    w_cps[1].start()
    x_cps[1].start()
    x_cps[0].wait()
    w_cps[0].start()
    w_cps[2].start()
    for c in x_cps[2:]:
        c.start()
    layernorm(0)
    w_cps[1].wait()
    x_cps[1].wait()
    kproj(0)
    layernorm(1)
    w_cps[0].wait()
    w_cps[2].wait()
    for c in x_cps[2:]:
        c.wait()
    for c in f_cps:
        c.start()
    wo_cp.start()
    wr16 = jnp.broadcast_to(wr_ref[...].reshape(1, D).astype(jnp.float32), (16, D))
    wqt = jnp.concatenate([wqkv_ref[0].astype(jnp.float32).T, wr16], axis=0).astype(jnp.bfloat16)
    wvt = wqkv_ref[2].astype(jnp.float32).T.astype(jnp.bfloat16)
    kproj(1)
    for qi in range(NQ):
        if qi + 2 < NQ:
            layernorm(qi + 2)
        qvproj(qi, wqt, wvt)
        if qi + 2 < NQ:
            kproj(qi + 2)

    st = {}

    def select_token():
        r = r_ref[...]
        rmax = jnp.max(r, axis=-1, keepdims=True)
        col = jax.lax.broadcasted_iota(jnp.int32, (8, S), 1)
        idx = jnp.min(jnp.where(r == rmax, col, S - 1))
        st["rmax"] = rmax[0:1]
        st["idx"] = idx
        blk = xn_ref[pl.ds(pl.multiple_of((idx // 16) * 16, 16), 16), :]
        rid = jax.lax.broadcasted_iota(jnp.int32, (16, D), 0)
        st["x_sel"] = jnp.where(rid == idx % 16, blk, jnp.zeros_like(blk))

    def gu_piece(j):
        cols = slice(j * FB, (j + 1) * FB)
        gate = jnp.dot(st["x_sel"], wg_ref[:, cols], preferred_element_type=jnp.float32)
        up = jnp.dot(st["x_sel"], wu_ref[:, cols], preferred_element_type=jnp.float32)
        st[("h", j)] = (gate * jax.nn.sigmoid(gate) * up).astype(jnp.bfloat16)

    def down_piece(j):
        y = jnp.dot(st[("h", j)], wd_ref[j * FB:(j + 1) * FB, :], preferred_element_type=jnp.float32)
        st["y"] = y if j == 0 else st["y"] + y
        if j == F // FB - 1:
            st["y1"] = jnp.sum(st["y"], axis=0, keepdims=True) * jax.nn.sigmoid(st["rmax"])

    ffn_pieces = ([functools.partial(gu_piece, j) for j in range(F // FB)]
                  + [functools.partial(down_piece, j) for j in range(F // FB)])

    o_cps = []

    def outproj(qi):
        ot = ot_ref[qi, 0:H].reshape(D, TQ)
        o = ot.T.astype(jnp.bfloat16)
        att = jnp.dot(o, wo_ref[...], preferred_element_type=jnp.float32)
        rows = slice(qi * TQ, (qi + 1) * TQ)
        rid = jax.lax.broadcasted_iota(jnp.int32, (TQ, D), 0) + qi * TQ
        upd = jnp.where(rid == st["idx"], st["y1"], 0.0)
        res = (x_ref[rows, :].astype(jnp.float32) + att) + (xn_ref[rows, :].astype(jnp.float32) + upd)
        o_ref[rows, :] = res.astype(o_ref.dtype)
        ocp = pltpu.make_async_copy(o_ref.at[pl.ds(qi * TQ, TQ)], o_hbm.at[pl.ds(qi * TQ, TQ)], sems.at[qi])
        ocp.start()
        o_cps.append(ocp)

    off_chunks = [c for c in range(NC) if (c * NOFF) // NC != ((c + 1) * NOFF) // NC]
    pieces = [(j, lt) for j in range(NOFF) for lt in range(NL)]

    def krows(h, r0, r1):
        return pltpu.bitcast(k_ref[h, r0 // 2:r1 // 2, :], jnp.bfloat16)

    def build_kb(h):
        for j, c in enumerate(off_chunks):
            kf = krows(h, c * CK + CK - 16, (c + 1) * CK).astype(jnp.float32)
            for d in range(Dh):
                kb_ref[d, j * 16:(j + 1) * 16, :] = jnp.broadcast_to(kf[:, d:d + 1], (16, 128))

    def build_qb(qi, h, qb_ref):
        qf = q_ref[qi, h].astype(jnp.float32)
        for d in range(Dh):
            qb_ref[d] = jnp.broadcast_to(qf[d:d + 1], (8, TQ))

    def piece(j, lt, s_ref, qb_ref):
        c = off_chunks[j]
        a = None
        for d in range(Dh):
            t_ = kb_ref[d, j * 16:(j + 1) * 16, :].reshape(2, 8, 128) * qb_ref[d, :, lt * 128:(lt + 1) * 128][None]
            a = t_ if a is None else a + t_
        s_ref[(c + 1) * CK - 16:(c + 1) * CK, lt * 128:(lt + 1) * 128] = a.reshape(16, 128)
        return jnp.maximum(a[0], a[1])

    def a_chunk(h, qm, c, s_ref, m):
        nrow = CK - 16 if c in off_chunks else CK
        s = jnp.dot(krows(h, c * CK, c * CK + nrow), qm, preferred_element_type=jnp.float32)
        s_ref[c * CK:c * CK + nrow, :] = s
        mc = jnp.max(s.reshape(nrow // 8, 8, TQ), axis=0)
        return (mc if m is None else jnp.maximum(m, mc)), s[0:8]

    def b_chunk(h, c, s_ref, m, acc, tok):
        m = jnp.broadcast_to(m, (8, TQ))
        if tok is not None:
            m = jnp.maximum(m, jnp.minimum(m, tok))
        p = jnp.exp2(s_ref[c * CK:(c + 1) * CK, :].reshape(CK // 8, 8, TQ) - m[None]).reshape(CK, TQ)
        l = None
        for kt in range(CK // 128):
            lt = None
            for r in reversed(range(8)):
                a = p[kt * 128 + r * 16: kt * 128 + r * 16 + 8] + p[kt * 128 + r * 16 + 8: kt * 128 + r * 16 + 16]
                lt = a if lt is None else lt + a
            l = lt if l is None else l + lt
        pv = jnp.dot(vt_ref[h, :, c * CK:(c + 1) * CK], p.astype(jnp.bfloat16), preferred_element_type=jnp.float32)
        return (pv, l) if acc is None else (acc[0] + pv, acc[1] + l)

    s_refs = (s0_ref, s1_ref)
    m_refs = (m0_ref, m1_ref)
    qb_refs = (qb0_ref, qb1_ref)

    def finish_b(acc, qi, hslot):
        o = acc[0] / jnp.sum(acc[1], axis=0, keepdims=True)
        ot_ref[qi, hslot] = o

    def head_iter(h, carry):
        hn = jnp.minimum(h + 1, H - 1)
        hp = jnp.maximum(h - 1, 0)
        hp_slot = jnp.where(h == 0, H, h - 1)
        qcache, pmax, binfo, acc, toks = {}, {}, {}, {}, []
        for i in range(NQ * NC):
            u, c = (SKEW + i) // NC, (SKEW + i) % NC
            ha = h if u < NQ else hn
            if u not in qcache:
                qcache[u] = q_ref[u % NQ, ha]
                pmax[u] = pm_ref[...] if c > 0 else None
            pmax[u], tk = a_chunk(ha, qcache[u], c, s_refs[u % 2], pmax[u])
            toks.append(tk)
            if NOFF and u < NQ:
                c_hi = PC_LAST if u == NQ - 1 else PC_HI
                nslot = c_hi - PC_LO + 1
                for pi, (j, lt) in enumerate(pieces):
                    if PC_LO + (pi * nslot) // len(pieces) == c:
                        v = piece(j, lt, s_refs[u % 2], qb_refs[u % 2])
                        ml = [pmax[u][:, i_ * 128:(i_ + 1) * 128] for i_ in range(NL)]
                        ml[lt] = jnp.maximum(ml[lt], v)
                        pmax[u] = jnp.concatenate(ml, axis=1)
                if c == QB_AT:
                    build_qb((u + 1) % NQ, h if u + 1 < NQ else hn, qb_refs[(u + 1) % 2])
                if u == NQ - 1 and c == PC_LAST + 1:
                    build_kb(hn)
            if c == NC - 1:
                m_refs[u % 2][...] = jnp.max(pmax[u], axis=0, keepdims=True)
            elif i == NQ * NC - 1:
                pm_ref[...] = pmax[u]
            u, c = i // NC - 1, i % NC
            if u not in binfo:
                binfo[u] = m_refs[u % 2][...]
                acc[u] = None
            acc[u] = b_chunk(h if u >= 0 else hp, c, s_refs[u % 2], binfo[u], acc[u],
                             toks[i - LAG] if i - LAG >= 0 else None)
            if c == NC - 1:
                finish_b(acc[u], u % NQ, h if u >= 0 else hp_slot)
        return carry

    m1_ref[...] = jnp.zeros(m1_ref.shape, jnp.float32)
    if NOFF:
        build_kb(0)
        build_qb(0, 0, qb0_ref)
    pm0 = None
    for c in range(SKEW):
        pm0, _ = a_chunk(0, q_ref[0, 0], c, s0_ref, pm0)
    if SKEW:
        pm_ref[...] = pm0

    select_token()

    jax.lax.fori_loop(0, H, head_iter, 0)

    for c in f_cps:
        c.wait()
    wo_cp.wait()
    mb = m_refs[(NQ - 1) % 2][...]
    acc = None
    for c in range(NC):
        if c < len(ffn_pieces):
            ffn_pieces[c]()
        acc = b_chunk(H - 1, c, s_refs[(NQ - 1) % 2], mb, acc, None)
    for pc in ffn_pieces[NC:]:
        pc()
    finish_b(acc, NQ - 1, H - 1)
    for qi in range(NQ):
        outproj(qi)
    for c in o_cps:
        c.wait()


@jax.jit
def pallas_parallel_sum__softmax_full_mha__moe_arch_mod__prompt_kernel(
    A_x: jax.Array,
    A_wqkv: jax.Array,
    A_wo: jax.Array,
    B_x: jax.Array,
    B_w_r: jax.Array,
    B_w_gate: jax.Array,
    B_w_up: jax.Array,
    B_w_down: jax.Array,
):
    B, S, D = A_x.shape
    assert B == 1
    F = B_w_gate.shape[1]
    Dh = D // H
    bf = jnp.bfloat16
    vmem = pl.BlockSpec(memory_space=pltpu.VMEM)
    hbm = pl.BlockSpec(memory_space=pl.ANY)
    out = pl.pallas_call(
        _kernel,
        out_shape=jax.ShapeDtypeStruct((S, D), A_x.dtype),
        in_specs=[hbm, hbm, hbm, vmem, hbm, hbm, hbm],
        out_specs=hbm,
        scratch_shapes=[
            pltpu.VMEM((S, D), bf),
            pltpu.VMEM((3, D, D), bf),
            pltpu.VMEM((D, D), bf),
            pltpu.VMEM((S, D), bf),
            pltpu.VMEM((S, D), bf),
            pltpu.VMEM((S // TQ, H, Dh, TQ), bf),
            pltpu.VMEM((H, S // 2, Dh), jnp.uint32),
            pltpu.VMEM((H, Dh, S), bf),
            pltpu.VMEM((S, TQ), jnp.float32),
            pltpu.VMEM((S, TQ), jnp.float32),
            pltpu.VMEM((1, TQ), jnp.float32),
            pltpu.VMEM((1, TQ), jnp.float32),
            pltpu.VMEM((8, TQ), jnp.float32),
            pltpu.VMEM((S // TQ, H + 1, Dh, TQ), jnp.float32),
            pltpu.VMEM((8, S), jnp.float32),
            pltpu.VMEM((Dh, max(NOFF, 1) * 16, 128), jnp.float32),
            pltpu.VMEM((Dh, 8, TQ), jnp.float32),
            pltpu.VMEM((Dh, 8, TQ), jnp.float32),
            pltpu.VMEM((D, F), bf),
            pltpu.VMEM((D, F), bf),
            pltpu.VMEM((F, D), bf),
            pltpu.SemaphoreType.DMA((7 + S // TQ,)),
        ],
        compiler_params=pltpu.CompilerParams(vmem_limit_bytes=100 * 1024 * 1024),
    )(A_x.reshape(S, D), A_wqkv, A_wo, B_w_r, B_w_gate, B_w_up, B_w_down)
    return out.reshape(B, S, D)
```
